```python
import os as _os
_os.environ.setdefault("JAX_PLATFORMS", "cpu")
import jax
import jax.numpy as jnp

def _softmax(x, axis=-1):
    return jax.nn.softmax(x, axis=axis)
def _gelu(x):
    return jax.nn.gelu(x, approximate=True)
def _silu(x):
    return jax.nn.silu(x)
def _sigmoid(x):
    return jax.nn.sigmoid(x)
def _layernorm(x, axis=-1, eps=1e-5):
    m = jnp.mean(x, axis=axis, keepdims=True)
    v = jnp.var(x, axis=axis, keepdims=True)
    return (x - m) / jnp.sqrt(v + eps)
def _scatter_add(tgt, idx, src, axis=0):
    return tgt.at[idx].add(src)
def _segment_sum(src, seg, n):
    return jax.ops.segment_sum(src, seg, n)
class _Rng:
    def __init__(self, key):
        self._k = key
    def _next(self):
        self._k, sub = jax.random.split(self._k)
        return sub
    def normal(self, shape):
        return jax.random.normal(self._next(), shape, dtype=jnp.bfloat16)
    def randint(self, lo, hi, shape):
        return jax.random.randint(self._next(), shape, lo, hi, dtype=jnp.int32)
    def uniform(self, shape, lo=0.0, hi=1.0):
        return jax.random.uniform(self._next(), shape, jnp.bfloat16, lo, hi)
    def permutation(self, n):
        return jax.random.permutation(self._next(), n)


kernel_name = 'gated_mix__compressed_kv_cla__ssm_conv_h3__prompt'

def setup_inputs():
    _rng = _Rng(jax.random.key(int.from_bytes(__import__("os").urandom(4), "little")))
    _w = (lambda a: (lambda t: t.astype(jnp.bfloat16) if jnp.issubdtype(t.dtype, jnp.floating) else t)(jnp.asarray(a)))
    def _A_setup():
        B, H, Sq, Sk, D, M = 1, 32, 2048, 2048, 128, 1024
        Dc = 4 * D
        return {
            "x": _w((lambda *s: _rng.normal(s) * 0.05)(B, Sq, M)),
            "c_kv": _w((lambda *s: _rng.normal(s) * 0.8)(B, Sk, Dc)),
            "w_q": _w((lambda *s: _rng.normal(s) * 3.2)(M, H, D) * (M ** -0.5)),
            "w_uk": _w((lambda *s: _rng.normal(s) * 3.2)(Dc, H, D) * (Dc ** -0.5)),
            "w_uv": _w((lambda *s: _rng.normal(s) * 0.8)(Dc, H, D) * (Dc ** -0.5)),
            "w_o": _w((lambda *s: _rng.normal(s) * 0.8)(H, D, M) * ((H * D) ** -0.5)),
        }
    _A_in = _A_setup()

    def _B_setup():
        B, S, D = 1, 2048, 1024
        ks = 4
        return {
            "q": _w((lambda *s: _rng.normal(s) * 0.05)(B, S, D)),
            "k": _w((lambda *s: _rng.normal(s) * 0.8)(B, S, D)),
            "v": _w((lambda *s: _rng.normal(s) * 0.8)(B, S, D)),
            "shift_k": _w((lambda *s: _rng.normal(s) * 0.8)(D, ks) * 0.5),
            "ssm_k": _w((lambda *s: _rng.normal(s) * 0.8)(D, S) * (1.0 / S ** 0.5)),
            "ssm_D": _w((lambda *s: _rng.normal(s) * 0.8)(D)),
        }
    _B_in = _B_setup()

    return {
        "A_x": _A_in["x"],
        "A_c_kv": _A_in["c_kv"],
        "A_w_q": _A_in["w_q"],
        "A_w_uk": _A_in["w_uk"],
        "A_w_uv": _A_in["w_uv"],
        "A_w_o": _A_in["w_o"],
        "B_q": _B_in["q"],
        "B_k": _B_in["k"],
        "B_v": _B_in["v"],
        "B_shift_k": _B_in["shift_k"],
        "B_ssm_k": _B_in["ssm_k"],
        "B_ssm_D": _B_in["ssm_D"],
        "gate_w": _w((lambda *s: _rng.normal(s) * 0.05)(1024) * 16.0),
    }

def reference(A_x, A_c_kv, A_w_q, A_w_uk, A_w_uv, A_w_o, B_q, B_k, B_v, B_shift_k, B_ssm_k, B_ssm_D, gate_w):
    def _A_ref(x, c_kv, w_q, w_uk, w_uv, w_o):
        B, Sq, M = x.shape[0], x.shape[1], x.shape[2]
        Sk = c_kv.shape[1]
        H, D = w_q.shape[1], w_q.shape[2]
        q = jnp.einsum("bqm,mhd->bhqd", x, w_q)
        k = jnp.einsum("bkc,chd->bhkd", c_kv, w_uk)
        v = jnp.einsum("bkc,chd->bhkd", c_kv, w_uv)
        scores = jnp.einsum("bhqd,bhkd->bhqk", q, k) * (D ** -0.5)
        off = Sk - Sq
        qi = jnp.arange(Sq)[:, None]
        kj = jnp.arange(Sk)[None, :]
        cmask = kj <= (qi + off)
        scores = jnp.where(cmask[None, None], scores, -1e9)
        p = _softmax(scores, axis=-1)
        ctx = jnp.einsum("bhqk,bhkd->bhqd", p, v)
        return jnp.einsum("bhqd,hdm->bqm", ctx, w_o)

    def _B_ref(q, k, v, shift_k, ssm_k, ssm_D):
        B, S, D = q.shape
        ks = shift_k.shape[-1]
        k_pad = jnp.pad(k, ((0, 0), (ks - 1, 0), (0, 0)))
        k_shift = jnp.zeros_like(k)
        for t in range(ks):
            k_shift = k_shift + k_pad[:, t:t + S, :] * shift_k[:, ks - 1 - t][None, None, :]
        kv = k_shift * v
        L = 2 * S
        kv_pad = jnp.pad(kv, ((0, 0), (0, S), (0, 0)))
        kf_pad = jnp.pad(ssm_k, ((0, 0), (0, S)))
        kv_f = (lambda x, axes=(-2,-1): jnp.fft.rfft2(x.astype(jnp.float32), axes=axes))(kv_pad[:, None, :, :], axes=(1, 2))
        kf_f = (lambda x, axes=(-2,-1): jnp.fft.rfft2(x.astype(jnp.float32), axes=axes))(kf_pad[:, None, :], axes=(1, 2))
        kf_f = (lambda x, *d: x.transpose(*d))(kf_f, 1, 2, 0)
        y_f = kv_f * kf_f[None, :, :, :]
        y = (lambda x, s, axes=(-2,-1): jnp.fft.irfft2(x, s=s, axes=axes).astype(jnp.bfloat16))(y_f, (1, L), axes=(1, 2))[:, 0, :S, :]
        y = y + kv * ssm_D[None, None, :]
        return q * y

    x = A_x
    g = _sigmoid((x * gate_w).sum(-1, keepdims=True))
    a = _A_ref(x, A_c_kv, A_w_q, A_w_uk, A_w_uv, A_w_o)
    b = _B_ref(x, B_k, B_v, B_shift_k, B_ssm_k, B_ssm_D)
    return g * a + (1 - g) * b
```

```python
import math

import jax
import jax.numpy as jnp
from jax import lax
from jax.experimental import pallas as pl
from jax.experimental.pallas import tpu as pltpu

BF16 = jnp.bfloat16
F32 = jnp.float32
U32 = jnp.uint32

LANES = 128
CHUNK = 128
BQ = 256
NEG = -1e30

_NT = (((1,), (1,)), ((), ()))


def _dot(a, b):
    return jnp.dot(a, b, preferred_element_type=F32)


def _dot_nt(a, b):
    return lax.dot_general(a, b, _NT, preferred_element_type=F32)


def _split_head_pair(raw_ref):
    half = raw_ref.shape[0] // 2
    a = raw_ref[pl.ds(0, half, stride=2), :]
    b = raw_ref[pl.ds(1, half, stride=2), :]
    lo = (a & U32(0xFFFF)) | (b << 16)
    hi = (a >> 16) | (b & U32(0xFFFF0000))
    return jnp.concatenate([pltpu.bitcast(lo, BF16), pltpu.bitcast(hi, BF16)], axis=1)


def _dft_matrices():
    c = CHUNK

    def angle(shape, fdim, tdim):
        slot = lax.broadcasted_iota(jnp.int32, shape, fdim)
        t = lax.broadcasted_iota(jnp.int32, shape, tdim)
        k = slot & (c - 1)
        f = jnp.where(k < c // 2, 2 * k, 2 * k - (c - 1))
        n = ((2 * f + 1) * t + jnp.where(slot >= c, c, 0)) & (4 * c - 1)
        n = jnp.where(n > 2 * c, 4 * c - n, n)
        return jnp.cos(n.astype(F32) * (math.pi / (2 * c)))

    fwd = angle((2 * c, c), 0, 1)
    inv = angle((c, 2 * c), 1, 0) * (1.0 / c)
    return fwd.astype(BF16), inv.astype(BF16)


def _attention(q_ref, k_ref, v_ref, o_ref, seq):
    row = lax.broadcasted_iota(jnp.int32, (BQ, BQ), 0)
    col = lax.broadcasted_iota(jnp.int32, (BQ, BQ), 1)
    causal = col <= row
    for i in range(seq // BQ):
        nk = (i + 1) * BQ
        s = _dot_nt(q_ref[i * BQ:nk, :], k_ref[0:nk, :])
        sd = jnp.where(causal, s[:, nk - BQ:], NEG)
        s = jnp.concatenate([s[:, :nk - BQ], sd], axis=1) if i else sd
        m = jnp.max(s, axis=1, keepdims=True)
        p = jnp.exp2(s - m)
        l = jnp.sum(p, axis=1, keepdims=True)
        o = _dot(p.astype(BF16), v_ref[0:nk, :])
        o_ref[i * BQ:nk, :] = (o * (1.0 / l)).astype(BF16)


def _kernel(x_hbm, c_hbm, wq_hbm, wk_hbm, wv_hbm, wo_hbm, bk_hbm, bv_hbm, hk_hbm,
            sh_ref, dd_ref, gw_ref,
            out_hbm,
            x_v, c_v, wq_raw, wk_raw, wv_raw, q_s, k_s, v_s, ctx_s,
            wo_v, bk_v, bv_v, hk_v, out_v, g_s, fwd_s, inv_s, par_s,
            kpad_s, kv_s, u_s, h_s, y_s,
            sem_in, sem_w, sem_b, sem_o):
    seq, dm = x_v.shape
    n_pairs = wq_hbm.shape[1]
    n_cb = dm // LANES
    n_ch = seq // CHUNK
    head_dim = wq_hbm.shape[-1]
    q_scale = head_dim ** -0.5 * math.log2(math.e)

    wq32, wk32, wv32 = (w.bitcast(U32) for w in (wq_hbm, wk_hbm, wv_hbm))

    def w_copies(j, slot):
        return (pltpu.make_async_copy(wk32.at[:, j, 0], wk_raw.at[slot], sem_w.at[0, slot]),
                pltpu.make_async_copy(wv32.at[:, j, 0], wv_raw.at[slot], sem_w.at[1, slot]),
                pltpu.make_async_copy(wq32.at[:, j, 0], wq_raw.at[slot], sem_w.at[2, slot]))

    def b_copies(cb, slot):
        cols = pl.ds(pl.multiple_of(cb * LANES, LANES), LANES)
        return (pltpu.make_async_copy(wo_hbm.at[:, cols], wo_v.at[slot], sem_b.at[0, slot]),
                pltpu.make_async_copy(bk_hbm.at[:, cols], bk_v.at[slot], sem_b.at[1, slot]),
                pltpu.make_async_copy(bv_hbm.at[:, cols], bv_v.at[slot], sem_b.at[2, slot]),
                pltpu.make_async_copy(hk_hbm.at[cols, :], hk_v.at[slot], sem_b.at[3, slot]))

    def out_copy(cb, slot):
        cols = pl.ds(pl.multiple_of(cb * LANES, LANES), LANES)
        return pltpu.make_async_copy(out_v.at[slot], out_hbm.at[:, cols], sem_o.at[slot])

    c_copy = pltpu.make_async_copy(c_hbm, c_v, sem_in.at[0])
    x_copy = pltpu.make_async_copy(x_hbm, x_v, sem_in.at[1])
    c_copy.start()
    for cp in w_copies(0, 0):
        cp.start()
    x_copy.start()

    fwd, inv = _dft_matrices()
    fwd_s[...] = fwd
    inv_s[...] = inv
    kpad_s[0:8, :] = jnp.zeros((8, LANES), F32)
    sh = sh_ref[...].astype(F32)
    dd = dd_ref[...].astype(F32)
    for cb in range(n_cb):
        for t in range(sh.shape[0]):
            par_s[cb, t] = jnp.broadcast_to(sh[t:t + 1, cb * LANES:(cb + 1) * LANES], (8, LANES))
        par_s[cb, sh.shape[0]] = jnp.broadcast_to(dd[cb:cb + 1, :], (8, LANES))

    c_copy.wait()
    x_copy.wait()
    for cp in b_copies(0, 0):
        cp.start()

    gw = gw_ref[...].astype(F32)
    for r in range(seq // 256):
        rows = slice(r * 256, (r + 1) * 256)
        acc = None
        for cb in range(n_cb):
            t = x_v[rows, cb * LANES:(cb + 1) * LANES].astype(F32) * gw[cb:cb + 1, :]
            acc = t if acc is None else acc + t
        z = jnp.sum(acc, axis=1, keepdims=True)
        g_s[rows, :] = jnp.broadcast_to(jax.nn.sigmoid(z), (256, LANES))

    def pair_step(j, _):
        slot = j & 1
        for cp in w_copies(j, slot):
            cp.wait()

        @pl.when(j + 1 < n_pairs)
        def _():
            for cp in w_copies(j + 1, 1 - slot):
                cp.start()

        wk = _split_head_pair(wk_raw.at[slot])
        wv = _split_head_pair(wv_raw.at[slot])
        wq = _split_head_pair(wq_raw.at[slot])
        mb = 512
        for r in range(seq // mb):
            rows = slice(r * mb, (r + 1) * mb)
            c = c_v[rows, :]
            k2 = _dot(c, wk).astype(BF16)
            v2 = _dot(c, wv).astype(BF16)
            q2 = (_dot(x_v[rows, :], wq) * q_scale).astype(BF16)
            for h in range(2):
                lanes = slice(h * head_dim, (h + 1) * head_dim)
                k_s[h, rows, :] = k2[:, lanes]
                v_s[h, rows, :] = v2[:, lanes]
                q_s[h, rows, :] = q2[:, lanes]

        def head_step(h, _):
            _attention(q_s.at[h], k_s.at[h], v_s.at[h], ctx_s.at[2 * j + h], seq)

        lax.fori_loop(0, 2, head_step, None)

    lax.fori_loop(0, n_pairs, pair_step, None)

    half = CHUNK // 2

    def block_step(cb, _):
        slot = cb & 1
        for cp in b_copies(cb, slot):
            cp.wait()

        @pl.when(cb + 1 < n_cb)
        def _():
            for cp in b_copies(cb + 1, 1 - slot):
                cp.start()

        @pl.when(cb >= 2)
        def _():
            out_copy(cb - 2, slot).wait()

        taps = sh_ref.shape[0]
        fwd = fwd_s[...]
        kpad_s[8:, :] = bk_v[slot].astype(F32)
        tap = [jnp.tile(par_s[cb, t], (CHUNK // 8, 1)) for t in range(taps)]
        for j in range(n_ch):
            ks = None
            for t in range(taps):
                term = kpad_s[pl.ds(8 + j * CHUNK - t, CHUNK), :] * tap[t]
                ks = term if ks is None else ks + term
            kv = (ks * bv_v[slot, j * CHUNK:(j + 1) * CHUNK, :].astype(F32)).astype(BF16)
            kv_s[j * CHUNK:(j + 1) * CHUNK, :] = kv
            u_s[j] = _dot(fwd, kv)

        prev = None
        for d in range(n_ch):
            cur = _dot_nt(fwd, hk_v[slot, :, d * CHUNK:(d + 1) * CHUNK])
            if prev is None:
                h_s[d] = cur
            else:
                h_s[d, 0:half] = cur[0:half] - prev[CHUNK:CHUNK + half]
                h_s[d, half:CHUNK] = cur[half:CHUNK] + prev[CHUNK + half:]
                h_s[d, CHUNK:CHUNK + half] = cur[CHUNK:CHUNK + half] + prev[0:half]
                h_s[d, CHUNK + half:] = cur[CHUNK + half:] - prev[half:CHUNK]
            prev = cur

        fb = 16
        for f in range(CHUNK // fb):
            re = slice(f * fb, (f + 1) * fb)
            im = slice(CHUNK + f * fb, CHUNK + (f + 1) * fb)
            for i in range(n_ch):
                yr = yi = None
                for d in range(i + 1):
                    gr, gi = h_s[d, re], h_s[d, im]
                    ur, ui = u_s[i - d, re], u_s[i - d, im]
                    tr = gr * ur - gi * ui
                    ti = gr * ui + gi * ur
                    yr = tr if yr is None else yr + tr
                    yi = ti if yi is None else yi + ti
                y_s[i, re] = yr.astype(BF16)
                y_s[i, im] = yi.astype(BF16)

        inv = inv_s[...]
        mb = 256
        skip = jnp.tile(par_s[cb, taps], (mb // 8, 1))
        cols = pl.ds(pl.multiple_of(cb * LANES, LANES), LANES)
        for r in range(seq // mb):
            rows = slice(r * mb, (r + 1) * mb)
            ctx = jnp.concatenate([ctx_s[h, rows, :] for h in range(2 * n_pairs)], axis=1)
            a = _dot(ctx, wo_v[slot])
            y = jnp.concatenate(
                [_dot(inv, y_s[r * (mb // CHUNK) + t]) for t in range(mb // CHUNK)], axis=0)
            b = x_v[rows, cols].astype(F32) * (y + kv_s[rows, :].astype(F32) * skip)
            g = g_s[rows, :]
            out_v[slot, rows, :] = (g * a + (1.0 - g) * b).astype(BF16)

        out_copy(cb, slot).start()

    lax.fori_loop(0, n_cb, block_step, None)
    out_copy(n_cb - 2, (n_cb - 2) & 1).wait()
    out_copy(n_cb - 1, (n_cb - 1) & 1).wait()


@jax.jit
def pallas_gated_mix__compressed_kv_cla__ssm_conv_h3__prompt_kernel(
    A_x: jax.Array,
    A_c_kv: jax.Array,
    A_w_q: jax.Array,
    A_w_uk: jax.Array,
    A_w_uv: jax.Array,
    A_w_o: jax.Array,
    B_q: jax.Array,
    B_k: jax.Array,
    B_v: jax.Array,
    B_shift_k: jax.Array,
    B_ssm_k: jax.Array,
    B_ssm_D: jax.Array,
    gate_w: jax.Array,
):
    del B_q
    batch, seq, dm = A_x.shape
    dc = A_c_kv.shape[-1]
    heads, hd = A_w_q.shape[1:]
    taps = B_shift_k.shape[-1]
    assert batch == 1 and A_c_kv.shape[1] == seq and hd == LANES and heads % 2 == 0
    n_cb = dm // LANES
    n_ch = seq // CHUNK

    hbm = pl.BlockSpec(memory_space=pl.ANY)
    vmem = pl.BlockSpec(memory_space=pltpu.VMEM)
    out = pl.pallas_call(
        _kernel,
        out_shape=jax.ShapeDtypeStruct((seq, dm), BF16),
        in_specs=[hbm] * 9 + [vmem] * 3,
        out_specs=hbm,
        scratch_shapes=[
            pltpu.VMEM((seq, dm), BF16),
            pltpu.VMEM((seq, dc), BF16),
            pltpu.VMEM((2, dm, hd), U32),
            pltpu.VMEM((2, dc, hd), U32),
            pltpu.VMEM((2, dc, hd), U32),
            pltpu.VMEM((2, seq, hd), BF16),
            pltpu.VMEM((2, seq, hd), BF16),
            pltpu.VMEM((2, seq, hd), BF16),
            pltpu.VMEM((heads, seq, hd), BF16),
            pltpu.VMEM((2, heads * hd, LANES), BF16),
            pltpu.VMEM((2, seq, LANES), BF16),
            pltpu.VMEM((2, seq, LANES), BF16),
            pltpu.VMEM((2, LANES, seq), BF16),
            pltpu.VMEM((2, seq, LANES), BF16),
            pltpu.VMEM((seq, LANES), F32),
            pltpu.VMEM((2 * CHUNK, CHUNK), BF16),
            pltpu.VMEM((CHUNK, 2 * CHUNK), BF16),
            pltpu.VMEM((n_cb, taps + 1, 8, LANES), F32),
            pltpu.VMEM((seq + 8, LANES), F32),
            pltpu.VMEM((seq, LANES), BF16),
            pltpu.VMEM((n_ch, 2 * CHUNK, LANES), F32),
            pltpu.VMEM((n_ch, 2 * CHUNK, LANES), F32),
            pltpu.VMEM((n_ch, 2 * CHUNK, LANES), BF16),
            pltpu.SemaphoreType.DMA((2,)),
            pltpu.SemaphoreType.DMA((3, 2)),
            pltpu.SemaphoreType.DMA((4, 2)),
            pltpu.SemaphoreType.DMA((2,)),
        ],
        compiler_params=pltpu.CompilerParams(vmem_limit_bytes=100 * 1024 * 1024),
        name="gated_mix_cla_h3",
    )(
        A_x.reshape(seq, dm),
        A_c_kv.reshape(seq, dc),
        A_w_q.reshape(dm, heads // 2, 2, hd),
        A_w_uk.reshape(dc, heads // 2, 2, hd),
        A_w_uv.reshape(dc, heads // 2, 2, hd),
        A_w_o.reshape(heads * hd, dm),
        B_k.reshape(seq, dm),
        B_v.reshape(seq, dm),
        B_ssm_k,
        B_shift_k.T,
        B_ssm_D.reshape(n_cb, LANES),
        gate_w.reshape(n_cb, LANES),
    )
    return out.reshape(batch, seq, dm)
```

```python
import math

import jax
import jax.numpy as jnp
import numpy as np
from jax import lax
from jax.experimental import pallas as pl
from jax.experimental.pallas import tpu as pltpu

BF16 = jnp.bfloat16
F32 = jnp.float32
U32 = jnp.uint32

LANES = 128
CHUNK = 128
TK = 128
BQ = 2 * TK
GROUP = 4
NEG = -1e30


def _dot(a, b):
    return jnp.dot(a, b, preferred_element_type=F32)


def _dot_nt(a, b):
    return lax.dot_general(a, b, (((1,), (1,)), ((), ())), preferred_element_type=F32)


def _load_rows(ref, r0, r1):
    return pltpu.bitcast(ref[r0 // 2:r1 // 2, :], BF16)


def _store_rows(ref, r0, val, base=0):
    ref[pl.ds(base + r0 // 2, val.shape[0] // 2), :] = pltpu.bitcast(val.astype(BF16), U32)


_USES = (((2, 1), (3, -1)), ((3, 1),), ((1, 1), (3, 1)), ((0, 1), (3, 1)),
         ((0, -1), (1, 1)), ((0, 1),), ((0, 1), (2, 1)))


def _left_operands(a11, a12, a21, a22):
    return (a21 + a22, a21 - a11, a11, a11 + a22, a11 + a12, a12 - a22, a22)


def _right_operands(b11, b12, b21, b22):
    return (b11, b11 + b12, b12 - b22, b11 + b22, b22, b21 + b22, b21 - b11)


def _accumulate(blocks, n, product):
    for c, sign in _USES[n]:
        if blocks[c] is None:
            blocks[c] = product if sign > 0 else (product,)
        elif isinstance(blocks[c], tuple):
            blocks[c] = product - blocks[c][0]
        else:
            blocks[c] = blocks[c] + product if sign > 0 else blocks[c] - product


def _head_pair_operands(raw_ref):
    half = raw_ref.shape[0] // 2
    quad = []
    for words in (raw_ref[0:half, :], raw_ref[half:, :]):
        quad += [pltpu.bitcast(words << 16, F32),
                 pltpu.bitcast(words & np.uint32(0xFFFF0000), F32)]
    return [t.astype(BF16) for t in _right_operands(*quad)]


def _dft_matrices():
    c = CHUNK

    def wave(f, t, imag):
        n = ((2 * f + 1) * t + jnp.where(imag, c, 0)) & (4 * c - 1)
        n = jnp.where(n > 2 * c, 4 * c - n, n)
        return jnp.cos(n.astype(F32) * (math.pi / (2 * c)))

    row = lax.broadcasted_iota(jnp.int32, (2 * c, c), 0)
    k = row & (c - 1)
    fwd = wave(jnp.where(k < c // 2, 2 * k, 2 * c - 1 - 2 * k),
               lax.broadcasted_iota(jnp.int32, (2 * c, c), 1), row >= c)
    row = lax.broadcasted_iota(jnp.int32, (c, c), 0)
    col = lax.broadcasted_iota(jnp.int32, (c, c), 1)
    inv = wave(2 * (col & (c // 2 - 1)),
               jnp.where(row < c // 2, 2 * row, 2 * row - (c - 1)), col >= c // 2)
    return fwd.astype(BF16), (inv * (1.0 / c)).astype(BF16)


def _scores(q, k_ref, r0, causal):
    upper = _dot_nt(q, _load_rows(k_ref, 0, r0 + TK))
    corner = _dot_nt(q[TK:], _load_rows(k_ref, r0 + TK, r0 + BQ))
    top = [jnp.where(causal, upper[:TK, r0:], NEG)]
    if r0:
        top.insert(0, upper[:TK, :r0])
    bottom = [upper[TK:], jnp.where(causal, corner, NEG)]
    strips = [jnp.concatenate(s, axis=1) for s in (top, bottom)]
    return [(s, jnp.max(s, axis=1, keepdims=True)) for s in strips]


def _softmax_times_v(strips, v_ref, r0):
    top, bottom = (jnp.exp2(s - m) for s, m in strips)
    upper = _dot(jnp.concatenate([top, bottom[:, :r0 + TK]], axis=0).astype(BF16),
                 _load_rows(v_ref, 0, r0 + TK))
    corner = _dot(bottom[:, r0 + TK:].astype(BF16), _load_rows(v_ref, r0 + TK, r0 + BQ))
    res = []
    for p, o in ((top, upper[:TK]), (bottom, upper[TK:] + corner)):
        l = jnp.sum(p, axis=1, keepdims=True)
        r = pltpu.reciprocal(l, approx=True)
        res.append(o * (r * (2.0 - l * r)))
    return res


def _kernel(x_hbm, c_hbm, wq_hbm, wk_hbm, wv_hbm, wo_hbm, bk_hbm, bv_hbm, hk_hbm,
            sh_hbm, dd_hbm, gw_hbm,
            out_hbm,
            x_v, c_v, xs_s, cs_s, wq_raw, wk_raw, wv_raw, att_s,
            wo_v, bk_v, bv_v, hk_v, out_v, fwd_s, inv_s, par_s, spec_s,
            sh_v, dd_v, gw_v, zero_s,
            sem_p, sem_in, sem_w, sem_b, sem_o):
    seq, dm = x_v.shape
    n_pairs = wq_hbm.shape[1]
    head_dim = wq_hbm.shape[-1]
    taps = sh_v.shape[0]
    n_cb = dm // LANES
    n_ch = seq // CHUNK
    n_qb = seq // BQ
    n_parts = sem_o.shape[1]
    q_scale = head_dim ** -0.5 * math.log2(math.e)
    kv_base = 7 * n_pairs // 2
    g_base = kv_base + 8

    wq32, wk32, wv32 = (w.bitcast(U32) for w in (wq_hbm, wk_hbm, wv_hbm))

    def kv_copies(j):
        return [pltpu.make_async_copy(src.at[:, j + p, 0], dst.at[p], sem_w.at[i, p])
                for p in range(2) for i, (src, dst) in enumerate(((wk32, wk_raw), (wv32, wv_raw)))]

    def q_copy(j):
        return pltpu.make_async_copy(wq32.at[:, j, 0], wq_raw.at[j & 1], sem_w.at[2, j & 1])

    def block_copies(cb):
        slot = cb & 1
        own, other = (pl.ds(pl.multiple_of(c * LANES, LANES), LANES) for c in (cb, cb ^ 1))
        rows = pl.ds(pl.multiple_of(slot * wo_v.shape[2], wo_v.shape[2]), wo_v.shape[2])
        return (pltpu.make_async_copy(wo_hbm.at[rows, own], wo_v.at[slot, 0], sem_b.at[0, slot]),
                pltpu.make_async_copy(wo_hbm.at[rows, other], wo_v.at[slot, 1], sem_b.at[1, slot]),
                pltpu.make_async_copy(bk_hbm.at[:, own], bk_v.at[slot], sem_b.at[2, slot]),
                pltpu.make_async_copy(bv_hbm.at[:, own], bv_v.at[slot], sem_b.at[3, slot]),
                pltpu.make_async_copy(hk_hbm.at[own, :], hk_v.at[slot], sem_b.at[4, slot]))

    def out_copy(s, part):
        rows = pl.ds(part * (seq // n_parts), seq // n_parts)
        cols = pl.ds(pl.multiple_of(s * 2 * LANES, 2 * LANES), 2 * LANES)
        return pltpu.make_async_copy(
            out_v.at[s & 1, rows], out_hbm.at[rows, cols], sem_o.at[s & 1, part])

    n_cc = sem_in.shape[0] - 1
    c_rows = [pl.ds(i * (seq // n_cc), seq // n_cc) for i in range(n_cc)]
    c_copies = [pltpu.make_async_copy(c_hbm.at[r], c_v.at[r], sem_in.at[1 + i])
                for i, r in enumerate(c_rows)]
    x_copy = pltpu.make_async_copy(x_hbm, x_v, sem_in.at[0])
    small = [pltpu.make_async_copy(src, dst, sem_p.at[i]) for i, (src, dst) in
             enumerate(((sh_hbm, sh_v), (dd_hbm, dd_v), (gw_hbm, gw_v)))]
    for cp in (*small, *c_copies, *kv_copies(0)):
        cp.start()

    fwd_s[...], inv_s[...] = _dft_matrices()
    spec_s[3 * n_ch:4 * n_ch] = jnp.zeros((n_ch, 2 * CHUNK, LANES), F32)
    zero_s[0] = 0
    for cp in small:
        cp.wait()
    sh = sh_v[...].astype(F32)
    dd = dd_v[...].astype(F32)
    for cb in range(n_cb):
        for t in range(taps):
            par_s[cb, t] = jnp.broadcast_to(sh[t:t + 1, cb * LANES:(cb + 1) * LANES], (8, LANES))
        par_s[cb, taps] = jnp.broadcast_to(dd[cb:cb + 1, :], (8, LANES))

    def split_rows(src_ref, dst_ref, b):
        half = src_ref.shape[1] // 2
        for r in range(0, TK, 16):
            quad = [src_ref[b * BQ + i * TK + r:b * BQ + i * TK + r + 16,
                            k * half:(k + 1) * half].astype(F32)
                    for i in range(2) for k in range(2)]
            for n, op in enumerate(_left_operands(*quad)):
                dst_ref[n, b * TK + r:b * TK + r + 16, :] = op.astype(BF16)

    for i, cp in enumerate(c_copies):
        cp.wait()
        if i == n_cc - 1:
            x_copy.start()
            q_copy(0).start()
        for b in range(i * n_qb // n_cc, (i + 1) * n_qb // n_cc):
            split_rows(c_v, cs_s, b)

    def kv_refs(p):
        return [[att_s.at[kv_base + 4 * p + 2 * i + h] for h in range(2)] for i in range(2)]

    def project_kv(p):
        wk, wv = (_head_pair_operands(w.at[p]) for w in (wk_raw, wv_raw))
        for b0 in range(0, n_qb, 2):
            kb, vb = [None] * 4, [None] * 4
            for n in range(7):
                left = cs_s[n, b0 * TK:(b0 + 2) * TK, :]
                _accumulate(kb, n, _dot(left, wk[n]))
                _accumulate(vb, n, _dot(left, wv[n]))
            for refs, blocks in zip(kv_refs(p), (kb, vb)):
                for c, val in enumerate(blocks):
                    for b in range(2):
                        _store_rows(refs[c % 2], (b0 + b) * BQ + (c // 2) * TK,
                                    val[b * TK:(b + 1) * TK])

    def gate(j):
        n_rows = seq // n_pairs
        rows = pl.ds(pl.multiple_of(j * n_rows, n_rows), n_rows)
        gw = gw_v[...].astype(F32)
        z = None
        for cb in range(n_cb):
            t = x_v[rows, cb * LANES:(cb + 1) * LANES].astype(F32) * gw[cb:cb + 1, :]
            z = t if z is None else z + t
        g = jnp.broadcast_to(jax.nn.sigmoid(jnp.sum(z, axis=1, keepdims=True)), (n_rows, LANES))
        per = att_s.shape[1] // n_rows
        att_s[g_base + j // per, pl.ds(pl.multiple_of(j % per * n_rows, n_rows), n_rows), :] = (
            pltpu.bitcast(g, U32))

    def attend_pair(j):
        wq = _head_pair_operands(wq_raw.at[j & 1])
        k_refs, v_refs = kv_refs(j & 1)
        causal = (lax.broadcasted_iota(jnp.int32, (TK, TK), 1)
                  <= lax.broadcasted_iota(jnp.int32, (TK, TK), 0))
        partial, q, strips, outs = {}, {}, {}, {}
        todo = [(b, n) for b in range(n_qb - 1, -1, -1) for n in range(7)]

        def project_q(count):
            for b, n in [todo.pop(0) for _ in range(count)]:
                blocks = partial.setdefault(b, [None] * 4)
                _accumulate(blocks, n, _dot(xs_s[n, b * TK:(b + 1) * TK, :], wq[n]))
                if n == 6:
                    q[b] = [(jnp.concatenate([blocks[h], blocks[2 + h]], axis=0)
                             * q_scale).astype(BF16) for h in range(2)]

        def scores(b, h):
            strips[b, h] = _scores(q[b][h], k_refs[h], b * BQ, causal)

        def attend(b, h):
            outs[b, h] = _softmax_times_v(strips[b, h], v_refs[h], b * BQ)

        def keep(b, r0, r1):
            if b < n_qb:
                quad = [outs[b, h][i][r0:r1] for i in range(2) for h in range(2)]
                for n, op in enumerate(_left_operands(*quad)):
                    _store_rows(att_s.at[n * (n_pairs // 2) + (j >> 1)], b * TK + r0, op,
                                pl.multiple_of((j & 1) * (seq // 4), seq // 4))

        project_q(10)
        for b in range(n_qb - 1, 1, -1):
            scores(b, 0)
            if b == n_qb - 1:
                gate(j)
            project_q(3 if n_qb - b <= 3 else 4)
            attend(b, 0)
            keep(b + 1, 0, 32)
            scores(b, 1)
            keep(b + 1, 32, 80)
            project_q(3)
            attend(b, 1)
            keep(b + 1, 80, TK)
        scores(1, 0)
        project_q(7)
        keep(2, 0, 32)
        scores(1, 1)
        attend(1, 0)
        keep(2, 32, 80)
        scores(0, 0)
        scores(0, 1)
        keep(2, 80, TK)
        attend(1, 1)
        attend(0, 0)
        attend(0, 1)
        keep(1, 0, TK)
        keep(0, 0, TK)

    def pair_step(j, _):
        @pl.when(j & 1 == 0)
        def _():
            for cp in kv_copies(j):
                cp.wait()
            project_kv(0)
            project_kv(1)

            @pl.when(j + 2 < n_pairs)
            def _():
                for cp in kv_copies(j + 2):
                    cp.start()

        @pl.when(j == 0)
        def _():
            x_copy.wait()
            for cp in (q_copy(1), *block_copies(0), *block_copies(1)):
                cp.start()
            for b in range(n_qb):
                split_rows(x_v, xs_s, b)

        q_copy(j).wait()
        attend_pair(j)

        @pl.when(j + 2 < n_pairs)
        def _():
            q_copy(j + 2).start()

    lax.fori_loop(0, n_pairs, pair_step, None)

    half = CHUNK // 2

    def block_step(cb, _):
        slot = cb & 1
        s = cb >> 1
        for cp in block_copies(cb):
            cp.wait()

        @pl.when(jnp.logical_and(slot == 0, s >= 2))
        def _():
            for part in range(n_parts):
                out_copy(s - 2, part).wait()

        zero = zero_s[0]
        fwd = fwd_s[...]
        kv, att = {}, {}

        def signal_spectrum(j):
            rows = slice(j * CHUNK, (j + 1) * CHUNK)
            cur = bk_v[slot, rows, :].astype(F32)
            before = (bk_v[slot, j * CHUNK - 16:j * CHUNK, :].astype(F32)[8:] if j
                      else jnp.zeros((8, LANES), F32))
            window = jnp.concatenate([before, cur], axis=0)
            shifted = None
            for t in range(taps):
                delayed = pltpu.roll(window, t, 0)[8:] if t else cur
                term = delayed * jnp.tile(par_s[cb, t], (CHUNK // 8, 1))
                shifted = term if shifted is None else shifted + term
            kv[j] = shifted * bv_v[slot, rows, :].astype(F32)
            spec_s[j] = _dot(fwd, kv[j].astype(BF16))

        def filter_spectrum(d, prev):
            cur = _dot_nt(fwd, hk_v[slot, :, d * CHUNK:(d + 1) * CHUNK])
            dst = spec_s.at[n_ch + d]
            if prev is None:
                dst[...] = cur
            else:
                dst[0:half] = cur[0:half] - prev[CHUNK:CHUNK + half]
                dst[half:CHUNK] = cur[half:CHUNK] + prev[CHUNK + half:]
                dst[CHUNK:CHUNK + half] = cur[CHUNK:CHUNK + half] + prev[0:half]
                dst[CHUNK + half:] = cur[CHUNK + half:] - prev[half:CHUNK]
            return cur

        def chunk_conv(i0):
            for f in range(0, CHUNK, 8):
                re, im = slice(f, f + 8), slice(CHUNK + f, CHUNK + f + 8)
                yr, yi, us = [None] * GROUP, [None] * GROUP, {}
                for d in range(i0 + GROUP):
                    gr, gi = spec_s[n_ch + d, re], spec_s[n_ch + d, im]
                    live = range(max(0, d - i0), GROUP)
                    for o in live:
                        j = i0 + o - d
                        if j not in us:
                            us[j] = spec_s[j, re], spec_s[j, im]
                        ur, ui = us[j]
                        if d == 0:
                            yr[o], yi[o] = gr * ur - gi * ui, gr * ui + gi * ur
                        else:
                            yr[o] = yr[o] + gr * ur - gi * ui
                            yi[o] = yi[o] + gr * ui + gi * ur
                    if d == i0 + GROUP - 1:
                        for o in range(GROUP):
                            spec_s[2 * n_ch + i0 + o, re] = yr[o]
                            spec_s[2 * n_ch + i0 + o, im] = yi[o]
                    yield 8 * len(live)

        def to_time(i):
            ar, br, ai, bi = (spec_s[2 * n_ch + i, h * half:(h + 1) * half] for h in range(4))
            even = jnp.concatenate([ar + br, ai - bi], axis=0).astype(BF16)
            odd = jnp.concatenate([ar - br, ai + bi], axis=0).astype(BF16)
            return _dot(inv_s[0:half, :], even), _dot(inv_s[half:, :], odd)

        def mix(i, r0, r1):
            rows = slice(i * CHUNK + r0, i * CHUNK + r1)
            acc = spec_s.at[3 * n_ch + i]
            per = att_s.shape[1] // CHUNK
            g = pltpu.bitcast(att_s[g_base + i // per,
                                    i % per * CHUNK + r0:i % per * CHUNK + r1, :], F32)
            skip = jnp.tile(par_s[cb, taps], ((r1 - r0) // 8, 1))
            cols = pl.ds(pl.multiple_of(cb * LANES, LANES), LANES)
            h3 = x_v[rows, cols].astype(F32) * (spec_s[2 * n_ch + i, r0:r1] + kv[i][r0:r1] * skip)
            own = (jnp.where(slot == 1, acc[CHUNK + r0:CHUNK + r1], 0.0)
                   + g * att[0, i][r0:r1] + (1.0 - g) * h3)
            other = jnp.where(slot == 1, acc[r0:r1], 0.0) + g * att[1, i][r0:r1]
            acc[r0:r1], acc[CHUNK + r0:CHUNK + r1] = own, other
            out_v[s & 1, rows, :] = jnp.concatenate([other, own], axis=1).astype(BF16)
            if rows.stop % (seq // n_parts) == 0:
                @pl.when(slot == 1)
                def _():
                    out_copy(s, rows.start // (seq // n_parts)).start()

        kg = 4
        n_k = n_pairs // 2 // kg
        right = []
        for k in range(n_k):
            quad = [jnp.concatenate(
                [wo_v[slot, c % 2, (2 * p + c // 2) * head_dim:(2 * p + c // 2 + 1) * head_dim, :]
                 for p in range(k * kg, (k + 1) * kg)], axis=0).astype(F32) for c in range(4)]
            right.append([t.astype(BF16) for t in _right_operands(*quad)])

        def project_out():
            for b in range(0, n_qb, 2):
                blocks = [None] * 4
                for n in range(7):
                    acc = None
                    for k in range(n_k):
                        left = jnp.concatenate(
                            [_load_rows(att_s.at[n * (n_pairs // 2) + slot * (n_pairs // 4) + p // 2],
                                        p % 2 * (seq // 2) + b * TK,
                                        p % 2 * (seq // 2) + (b + 2) * TK)
                             for p in range(k * kg, (k + 1) * kg)], axis=1)
                        part = _dot(left, right[k][n])
                        acc = part if acc is None else acc + part
                        if k + 1 == n_k:
                            _accumulate(blocks, n, acc)
                            if n == 6:
                                for c, val in enumerate(blocks):
                                    for i in range(2):
                                        att[c % 2, 2 * (b + i) + c // 2] = val[i * TK:(i + 1) * TK]
                        yield part

        n_mm = (n_qb // 2) * 7 * n_k
        sub, mix_rows, delay, ahead = 8, 16, 3, 4
        n_paced = n_mm - delay - 1
        mix_cost, spectra_cost, weight_cost = 40, 400, 250
        total = (CHUNK * n_ch * (n_ch + 1) // 2 + n_ch * spectra_cost + 7 * n_k * weight_cost
                 + (n_ch - GROUP) * (CHUNK // mix_rows) * mix_cost)
        prev = None
        for d in range(ahead):
            prev = filter_spectrum(d, prev)
        spent, i0, conv = 0, 0, chunk_conv(0)
        inverses, times, mixes = {}, [], []
        matmuls = project_out()
        for t in range(n_mm):
            projected = set(att)
            part = next(matmuls)
            if t < 7 * n_k:
                spent += weight_cost
            if t < n_ch:
                if t + ahead < n_ch:
                    prev = filter_spectrum(t + ahead, prev)
                signal_spectrum(t)
                spent += spectra_cost
            for i, (even, odd) in times:
                spec_s[2 * n_ch + i, pl.ds(0, half, stride=2), :] = even
                spec_s[2 * n_ch + i, pl.ds(1, half, stride=2), :] = odd
                mixes += [(i, r, r + mix_rows) for r in range(0, CHUNK, mix_rows)]
            times = [(i, to_time(i)) for i in inverses.pop(t, ())]
            have = min(max(t - 1, 0), n_ch)
            for u in range(sub if t < n_paced and have >= GROUP else 0):
                r0 = u * (part.shape[0] // sub)
                spec_s[zero + 4 * n_ch, 0:8] = part[r0:r0 + 8]
                if mixes and (0, mixes[0][0]) in projected:
                    mix(*mixes.pop(0))
                    spent += mix_cost
                last = (t + 1, u + 1) == (n_paced, sub)
                while (conv and have >= i0 + GROUP
                       and (last or spent * n_paced * sub < total * (t * sub + u + 1))):
                    cost = next(conv, None)
                    if cost is None:
                        inverses.setdefault(t + delay, []).extend(range(i0, i0 + GROUP))
                        i0 += GROUP
                        conv = chunk_conv(i0) if i0 < n_ch else None
                    else:
                        spent += cost
        assert not (times or inverses or conv)
        for m in mixes:
            mix(*m)

        @pl.when(cb + 2 < n_cb)
        def _():
            for cp in block_copies(cb + 2):
                cp.start()

    lax.fori_loop(0, n_cb, block_step, None)
    for s in (n_cb // 2 - 2, n_cb // 2 - 1):
        for part in range(n_parts):
            out_copy(s, part).wait()


@jax.jit
def pallas_gated_mix__compressed_kv_cla__ssm_conv_h3__prompt_kernel(
    A_x: jax.Array,
    A_c_kv: jax.Array,
    A_w_q: jax.Array,
    A_w_uk: jax.Array,
    A_w_uv: jax.Array,
    A_w_o: jax.Array,
    B_q: jax.Array,
    B_k: jax.Array,
    B_v: jax.Array,
    B_shift_k: jax.Array,
    B_ssm_k: jax.Array,
    B_ssm_D: jax.Array,
    gate_w: jax.Array,
):
    del B_q
    batch, seq, dm = A_x.shape
    dc = A_c_kv.shape[-1]
    heads, hd = A_w_q.shape[1:]
    taps = B_shift_k.shape[-1]
    assert batch == 1 and A_c_kv.shape[1] == seq and hd == LANES and heads % 16 == 0 and taps <= 8
    n_cb = dm // LANES
    n_ch = seq // CHUNK

    hbm = pl.BlockSpec(memory_space=pl.ANY)
    out = pl.pallas_call(
        _kernel,
        out_shape=jax.ShapeDtypeStruct((seq, dm), BF16),
        in_specs=[hbm] * 12,
        out_specs=hbm,
        scratch_shapes=[
            pltpu.VMEM((seq, dm), BF16),
            pltpu.VMEM((seq, dc), BF16),
            pltpu.VMEM((7, seq // 2, dm // 2), BF16),
            pltpu.VMEM((7, seq // 2, dc // 2), BF16),
            pltpu.VMEM((2, dm, hd), U32),
            pltpu.VMEM((2, dc, hd), U32),
            pltpu.VMEM((2, dc, hd), U32),
            pltpu.VMEM((7 * heads // 4 + 10, seq // 2, hd), U32),
            pltpu.VMEM((2, 2, heads * hd // 2, LANES), BF16),
            pltpu.VMEM((2, seq, LANES), BF16),
            pltpu.VMEM((2, seq, LANES), BF16),
            pltpu.VMEM((2, LANES, seq), BF16),
            pltpu.VMEM((2, seq, 2 * LANES), BF16),
            pltpu.VMEM((2 * CHUNK, CHUNK), BF16),
            pltpu.VMEM((CHUNK, CHUNK), BF16),
            pltpu.VMEM((n_cb, taps + 1, 8, LANES), F32),
            pltpu.VMEM((4 * n_ch + 1, 2 * CHUNK, LANES), F32),
            pltpu.VMEM((taps, dm), BF16),
            pltpu.VMEM((n_cb, LANES), BF16),
            pltpu.VMEM((n_cb, LANES), BF16),
            pltpu.SMEM((1,), jnp.int32),
            pltpu.SemaphoreType.DMA((3,)),
            pltpu.SemaphoreType.DMA((5,)),
            pltpu.SemaphoreType.DMA((3, 2)),
            pltpu.SemaphoreType.DMA((5, 2)),
            pltpu.SemaphoreType.DMA((2, 4)),
        ],
        compiler_params=pltpu.CompilerParams(vmem_limit_bytes=110 * 1024 * 1024),
        name="gated_mix_cla_h3",
    )(
        A_x.reshape(seq, dm),
        A_c_kv.reshape(seq, dc),
        A_w_q.reshape(dm, heads // 2, 2, hd),
        A_w_uk.reshape(dc, heads // 2, 2, hd),
        A_w_uv.reshape(dc, heads // 2, 2, hd),
        A_w_o.reshape(heads * hd, dm),
        B_k.reshape(seq, dm),
        B_v.reshape(seq, dm),
        B_ssm_k,
        B_shift_k.T,
        B_ssm_D.reshape(n_cb, LANES),
        gate_w.reshape(n_cb, LANES),
    )
    return out.reshape(batch, seq, dm)
```
